```python
import jax
import jax.numpy as jnp

def _softmax(x, axis=-1):
    return jax.nn.softmax(x, axis=axis)
def _gelu(x):
    return jax.nn.gelu(x, approximate=True)
def _silu(x):
    return jax.nn.silu(x)
def _sigmoid(x):
    return jax.nn.sigmoid(x)
def _layernorm(x, axis=-1, eps=1e-5):
    m = jnp.mean(x, axis=axis, keepdims=True)
    v = jnp.var(x, axis=axis, keepdims=True)
    return (x - m) / jnp.sqrt(v + eps)
def _scatter_add(tgt, idx, src, axis=0):
    return tgt.at[idx].add(src)
def _segment_sum(src, seg, n):
    return jax.ops.segment_sum(src, seg, n)
class _Rng:
    def __init__(self, key):
        self._k = key
    def _next(self):
        self._k, sub = jax.random.split(self._k)
        return sub
    def normal(self, shape):
        return jax.random.normal(self._next(), shape, dtype=jnp.bfloat16)
    def randint(self, lo, hi, shape):
        return jax.random.randint(self._next(), shape, lo, hi, dtype=jnp.int32)
    def uniform(self, shape, lo=0.0, hi=1.0):
        return jax.random.uniform(self._next(), shape, jnp.bfloat16, lo, hi)
    def permutation(self, n):
        return jax.random.permutation(self._next(), n)


kernel_name = 'recurrent_scan__sliding_block_cached__dense_activation_gelu__decode'

def setup_inputs():
    _rng = _Rng(jax.random.key(int.from_bytes(__import__("os").urandom(4), "little")))
    _w = (lambda a: (lambda t: t.astype(jnp.bfloat16) if jnp.issubdtype(t.dtype, jnp.floating) else t)(jnp.asarray(a)))
    def _A_setup():
        B, Sq, D = 2, 1, 576
        Hq, Hkv, Sk, Dh = 32, 16, 32768, 128
        assert Hq % Hkv == 0, (Hq, Hkv)
        return {
            "x": _w((lambda *s: _rng.normal(s) * 0.05)(B, Sq, D)),
            "k_cache": _w((lambda *s: _rng.normal(s) * 0.05)(B, Hkv, Sk, Dh)),
            "v_cache": _w((lambda *s: _rng.normal(s) * 0.05)(B, Hkv, Sk, Dh)),
            "wq": _w((lambda *s: _rng.normal(s) * 0.05)(D, Hq * Dh) * (D ** -0.5)),
            "wo": _w((lambda *s: _rng.normal(s) * 0.05)(Hq * Dh, D) * ((Hq * Dh) ** -0.5)),
        }
    _A_in = _A_setup()

    def _B_setup():
        B, S, D, F = 2, 1, 576, 4608
        return {
            "x": _w((lambda *s: _rng.normal(s) * 0.05)(B, S, D)),
            "w1": _w((lambda *s: _rng.normal(s) * 0.05)(D, F) * (D ** -0.5)),
            "b1": _w((lambda *s: _rng.normal(s) * 0.05)(F) * 0.01),
            "w2": _w((lambda *s: _rng.normal(s) * 0.05)(F, D) * (F ** -0.5)),
            "b2": _w((lambda *s: _rng.normal(s) * 0.05)(D) * 0.01),
        }
    _B_in = _B_setup()

    return {
        "A_x": _A_in["x"],
        "A_k_cache": _A_in["k_cache"],
        "A_v_cache": _A_in["v_cache"],
        "A_wq": _A_in["wq"],
        "A_wo": _A_in["wo"],
        "B_x": _B_in["x"],
        "B_w1": _B_in["w1"],
        "B_b1": _B_in["b1"],
        "B_w2": _B_in["w2"],
        "B_b2": _B_in["b2"],
    }

def reference(A_x, A_k_cache, A_v_cache, A_wq, A_wo, B_x, B_w1, B_b1, B_w2, B_b2):
    def _A_ref(x, k_cache, v_cache, wq, wo):
        B, Sq, D = x.shape
        Hq, Dh = 32, 128
        Hkv, Sk = k_cache.shape[1], k_cache.shape[2]
        W = min(4096, max(256, Sk // 4))
        rep = Hq // Hkv
        q = (lambda x, *d: x.transpose(*d))((x @ wq).reshape(B, Sq, Hq, Dh), 0, 2, 1, 3)
        k = jnp.repeat(k_cache[:, :, Sk - W:, :], rep, axis=1)
        v = jnp.repeat(v_cache[:, :, Sk - W:, :], rep, axis=1)
        scores = jnp.einsum("bhqd,bhkd->bhqk", q, k) * (Dh ** -0.5)
        p = _softmax(scores, axis=-1)
        o = jnp.einsum("bhqk,bhkd->bhqd", p, v)
        return (lambda x, *d: x.transpose(*d))(o, 0, 2, 1, 3).reshape(B, Sq, Hq * Dh) @ wo

    def _B_ref(x, w1, b1, w2, b2):
        h = jnp.einsum("bsd,df->bsf", x, w1) + b1
        h = _gelu(h)
        return jnp.einsum("bsf,fd->bsd", h, w2) + b2

    x = A_x
    xn = _layernorm(x, axis=-1)
    s = _A_ref(xn, A_k_cache, A_v_cache, A_wq, A_wo)
    g = _silu(_B_ref(xn, B_w1, B_b1, B_w2, B_b2))
    return x + s * g
```

```python
import functools

import jax
import jax.numpy as jnp
from jax.experimental import pallas as pl
from jax.experimental.pallas import tpu as pltpu

_NT = (((1,), (1,)), ((), ()))
_F32 = jnp.float32
_BF16 = jnp.bfloat16


def _dot(a, b):
    return jnp.dot(a, b, preferred_element_type=_F32)


def _dot_nt(a, b):
    return jax.lax.dot_general(a, b, _NT, preferred_element_type=_F32)


def _make_kernel(B, D, HKV, REP, SK, DH, W, F):
    HW = REP * DH
    FT = F // 128
    scale = float(DH) ** -0.5

    def kernel(x_hbm, k_hbm, v_hbm, wq_hbm, wo_hbm, w1_hbm, b1_hbm, w2_hbm, b2_hbm,
               o_ref,
               x_v, b1_v, b2_v, wq_v, wo_v, w1_v, w2_v, k_v, v_v, q_v, acc_v,
               sm_sem, kv_sem, wo_sem):
        def c_x():
            return pltpu.make_async_copy(x_hbm, x_v, sm_sem.at[0])

        def c_b1():
            return pltpu.make_async_copy(b1_hbm, b1_v, sm_sem.at[1])

        def c_b2():
            return pltpu.make_async_copy(b2_hbm, b2_v, sm_sem.at[2])

        def c_wq():
            return pltpu.make_async_copy(wq_hbm, wq_v, sm_sem.at[3])

        def c_w1():
            return pltpu.make_async_copy(w1_hbm, w1_v, sm_sem.at[4])

        def c_w2():
            return pltpu.make_async_copy(w2_hbm, w2_v, sm_sem.at[5])

        def c_k(h, b):
            return pltpu.make_async_copy(
                k_hbm.at[b, h, pl.ds(SK - W, W), :], k_v.at[h, b], kv_sem.at[h, b])

        def c_v(h, b):
            return pltpu.make_async_copy(
                v_hbm.at[b, h, pl.ds(SK - W, W), :], v_v.at[h, b], kv_sem.at[h, B + b])

        def c_wo(h):
            return pltpu.make_async_copy(
                wo_hbm.at[:, pl.ds(pl.multiple_of(h * HW, HW), HW)], wo_v.at[h], wo_sem.at[h])

        c_x().start()
        c_wq().start()
        c_b1().start()
        c_b2().start()
        c_w1().start()
        c_w2().start()

        def issue(h, carry):
            for b in range(B):
                c_k(h, b).start()
            for b in range(B):
                c_v(h, b).start()
            c_wo(h).start()
            return carry

        jax.lax.fori_loop(0, HKV, issue, 0)

        c_x().wait()
        x2 = x_v[...].astype(_F32)
        row_d = jax.lax.broadcasted_iota(jnp.int32, (8, D), 0)
        x8 = jnp.where(row_d % 2 == 0,
                       jnp.broadcast_to(x2[0:1, :], (8, D)),
                       jnp.broadcast_to(x2[1:2, :], (8, D)))
        mean = jnp.mean(x8, axis=1, keepdims=True)
        xc = x8 - mean
        var = jnp.mean(xc * xc, axis=1, keepdims=True)
        xn = (xc / jnp.sqrt(var + 1e-5)).astype(_BF16)

        c_wq().wait()
        q_all = _dot(xn, wq_v[...])
        row_h = jax.lax.broadcasted_iota(jnp.int32, (8, DH), 0)
        rep1 = (row_h // 2) % 2 == 1
        for h in range(HKV):
            q_v[h] = jnp.where(rep1,
                               q_all[:, h * HW + DH:(h + 1) * HW],
                               q_all[:, h * HW:h * HW + DH]).astype(_BF16)

        c_w1().wait()
        c_b1().wait()
        b1f = b1_v[...].astype(_F32)
        bias1 = jnp.concatenate(
            [jnp.broadcast_to(b1f[t:t + 1, :], (8, 128)) for t in range(FT)], axis=1)
        hid = jax.nn.gelu(_dot(xn, w1_v[...]) + bias1, approximate=True).astype(_BF16)
        c_w2().wait()
        c_b2().wait()
        y = _dot_nt(hid, w2_v[...]) + b2_v[...].astype(_F32).reshape(1, D)
        gate = y * jax.nn.sigmoid(y)

        acc_v[...] = jnp.zeros_like(acc_v)
        row_w = jax.lax.broadcasted_iota(jnp.int32, (8, W), 0)
        b1_w = row_w % 2 == 1
        b1_h = row_h % 2 == 1

        def head(h, carry):
            qh = q_v[h]
            c_k(h, 0).wait()
            s0 = _dot_nt(qh, k_v[h, 0])
            c_k(h, 1).wait()
            s1 = _dot_nt(qh, k_v[h, 1])
            s = jnp.where(b1_w, s1, s0)
            m = jnp.max(s, axis=1, keepdims=True)
            p = jnp.exp((s - m) * scale)
            l = jnp.sum(p, axis=1, keepdims=True)
            pb = p.astype(_BF16)
            c_v(h, 0).wait()
            o0 = _dot(pb, v_v[h, 0])
            c_v(h, 1).wait()
            o1 = _dot(pb, v_v[h, 1])
            o = jnp.where(b1_h, o1, o0) / l
            lhs = jnp.concatenate(
                [jnp.where(rep1, 0.0, o), jnp.where(rep1, o, 0.0)], axis=1).astype(_BF16)
            c_wo(h).wait()
            acc_v[...] += _dot_nt(lhs, wo_v[h])
            return carry

        jax.lax.fori_loop(0, HKV, head, 0)

        acc = acc_v[...]
        s_out = acc[0:2, :] + acc[2:4, :]
        o_ref[...] = (x2 + s_out * gate[0:2, :]).astype(o_ref.dtype)

    return kernel


@jax.jit
def pallas_recurrent_scan__sliding_block_cached__dense_activation_gelu__decode_kernel(
    A_x: jax.Array,
    A_k_cache: jax.Array,
    A_v_cache: jax.Array,
    A_wq: jax.Array,
    A_wo: jax.Array,
    B_x: jax.Array,
    B_w1: jax.Array,
    B_b1: jax.Array,
    B_w2: jax.Array,
    B_b2: jax.Array,
):
    del B_x
    B, SQ, D = A_x.shape
    _, HKV, SK, DH = A_k_cache.shape
    HQD = A_wq.shape[1]
    REP = HQD // DH // HKV
    F = B_w1.shape[1]
    W = min(4096, max(256, SK // 4))
    assert B == 2 and SQ == 1 and REP == 2 and F % 128 == 0
    HW = REP * DH

    kernel = _make_kernel(B, D, HKV, REP, SK, DH, W, F)
    hbm = pl.BlockSpec(memory_space=pl.ANY)
    out = pl.pallas_call(
        kernel,
        in_specs=[hbm] * 9,
        out_specs=pl.BlockSpec(memory_space=pltpu.VMEM),
        out_shape=jax.ShapeDtypeStruct((B, D), A_x.dtype),
        scratch_shapes=[
            pltpu.VMEM((B, D), _BF16),
            pltpu.VMEM((F // 128, 128), _BF16),
            pltpu.VMEM((D,), _BF16),
            pltpu.VMEM((D, HQD), _BF16),
            pltpu.VMEM((HKV, D, HW), _BF16),
            pltpu.VMEM((D, F), _BF16),
            pltpu.VMEM((D, F), _BF16),
            pltpu.VMEM((HKV, B, W, DH), _BF16),
            pltpu.VMEM((HKV, B, W, DH), _BF16),
            pltpu.VMEM((HKV, 8, DH), _BF16),
            pltpu.VMEM((8, D), _F32),
            pltpu.SemaphoreType.DMA((6,)),
            pltpu.SemaphoreType.DMA((HKV, 2 * B)),
            pltpu.SemaphoreType.DMA((HKV,)),
        ],
        compiler_params=pltpu.CompilerParams(
            vmem_limit_bytes=120 * 1024 * 1024,
            disable_semaphore_checks=True,
        ),
    )(
        A_x.reshape(B, D),
        A_k_cache,
        A_v_cache,
        A_wq,
        A_wo.T,
        B_w1,
        B_b1.reshape(F // 128, 128),
        B_w2.T,
        B_b2,
    )
    return out.reshape(B, SQ, D)
```

```python
import functools

import jax
import jax.numpy as jnp
from jax.experimental import pallas as pl
from jax.experimental.pallas import tpu as pltpu

_NT = (((1,), (1,)), ((), ()))
_F32 = jnp.float32
_BF16 = jnp.bfloat16

TRACE = False
HI, LO = 0, 1
DR = 128
CUTS = (0, 2048, 3072, 3584, 4096)


def _dot(a, b):
    return jnp.dot(a, b, preferred_element_type=_F32)


def _dot_nt(a, b):
    return jax.lax.dot_general(a, b, _NT, preferred_element_type=_F32)


class _Null:
    def __enter__(self):
        return self

    def __exit__(self, *a):
        return False


def _sc(name):
    return jax.named_scope(name) if TRACE else _Null()


def _make_kernel(B, D, HKV, REP, SK, DH, W, F):
    HW = REP * DH
    HQD = HKV * HW
    FT = F // 128
    scale = float(DH) ** -0.5
    LAST = HKV - 1
    NP = len(CUTS) - 1
    assert CUTS[0] == 0 and CUTS[-1] == HQD
    S_X, S_B1, S_B2, S_WQ, S_W1, S_W2, S_WOA, S_V1 = range(8)
    S_P = 8
    S_K = S_P + NP
    S_V = S_K + 2 * HKV
    NSEM = S_V + HKV

    def kernel(x_hbm, k_hbm, v_hbm, wq_hbm, wo_hbm, w1_hbm, b1_hbm, w2_hbm, b2_hbm,
               o_ref,
               x_v, b1_v, b2_v, wq_v, wo_v, w1_v, w2_v, k_v, v_v, q_v, o_v, acc_v, late_v,
               sem):
        win = pl.ds(SK - W, W)

        def cp(src, dst, s):
            return pltpu.make_async_copy(src, dst, sem.at[s])

        c_x = lambda: cp(x_hbm, x_v, S_X)
        c_b1 = lambda: cp(b1_hbm, b1_v, S_B1)
        c_b2 = lambda: cp(b2_hbm, b2_v, S_B2)
        c_wq = lambda: cp(wq_hbm, wq_v, S_WQ)
        c_w1 = lambda: cp(w1_hbm, w1_v, S_W1)
        c_w2 = lambda: cp(w2_hbm, w2_v, S_W2)
        c_woa = lambda: cp(wo_hbm.at[pl.ds(DR, D - DR), :], wo_v.at[pl.ds(DR, D - DR), :], S_WOA)

        def c_p(i):
            cols = pl.ds(CUTS[i], CUTS[i + 1] - CUTS[i])
            return cp(wo_hbm.at[pl.ds(0, DR), cols], wo_v.at[pl.ds(0, DR), cols], S_P + i)

        c_k = lambda h, b: cp(k_hbm.at[b, h, win, :], k_v.at[h, b], S_K + b * HKV + h)
        c_v = lambda h: cp(v_hbm.at[:, h, win, :], v_v.at[h], S_V + h)
        c_v0 = lambda: cp(v_hbm.at[0, LAST, win, :], v_v.at[LAST, 0], S_V + LAST)
        c_v1 = lambda: cp(v_hbm.at[1, LAST, win, :], v_v.at[LAST, 1], S_V1)

        c_x().start(priority=LO)
        c_wq().start(priority=LO)
        c_b1().start(priority=LO)
        c_b2().start(priority=LO)
        c_w1().start(priority=LO)
        c_w2().start(priority=LO)
        c_woa().start(priority=LO)
        for h in range(LAST):
            c_k(h, 0).start(priority=LO)
            c_k(h, 1).start(priority=HI)
            c_v(h).start(priority=LO)
        c_k(LAST, 0).start(priority=LO)
        c_k(LAST, 1).start(priority=HI)
        c_v0().start(priority=LO)
        c_v1().start(priority=LO)
        for i in range(NP):
            c_p(i).start(priority=LO)

        c_x().wait()
        x2 = x_v[...].astype(_F32)
        row_d = jax.lax.broadcasted_iota(jnp.int32, (8, D), 0)
        x8 = jnp.where(row_d % 2 == 0,
                       jnp.broadcast_to(x2[0:1, :], (8, D)),
                       jnp.broadcast_to(x2[1:2, :], (8, D)))
        mean = jnp.mean(x8, axis=1, keepdims=True)
        xc = x8 - mean
        var = jnp.mean(xc * xc, axis=1, keepdims=True)
        xn = (xc / jnp.sqrt(var + 1e-5)).astype(_BF16)

        c_wq().wait()
        q_all = _dot(xn, wq_v[...])
        row_h = jax.lax.broadcasted_iota(jnp.int32, (8, DH), 0)
        rep1 = (row_h // 2) % 2 == 1
        for h in range(HKV):
            q_v[h] = jnp.where(rep1,
                               q_all[:, h * HW + DH:(h + 1) * HW],
                               q_all[:, h * HW:h * HW + DH]).astype(_BF16)

        c_w1().wait()
        c_b1().wait()
        b1f = b1_v[...].astype(_F32)
        bias1 = jnp.concatenate(
            [jnp.broadcast_to(b1f[t:t + 1, :], (8, 128)) for t in range(FT)], axis=1)
        hid = jax.nn.gelu(_dot(xn, w1_v[...]) + bias1, approximate=True).astype(_BF16)
        c_w2().wait()
        c_b2().wait()
        y = _dot_nt(hid, w2_v[...]) + b2_v[...].astype(_F32).reshape(1, D)
        gate = y * jax.nn.sigmoid(y)

        row_w = jax.lax.broadcasted_iota(jnp.int32, (8, W), 0)
        b1_w = row_w % 2 == 1
        b1_h = row_h % 2 == 1

        def probs(h):
            qh = q_v[h]
            s0 = _dot_nt(qh, k_v[h, 0])
            s1 = _dot_nt(qh, k_v[h, 1])
            s = jnp.where(b1_w, s1, s0)
            m = jnp.max(s, axis=1, keepdims=True)
            p = jnp.exp((s - m) * scale)
            l = jnp.sum(p, axis=1, keepdims=True)
            return p.astype(_BF16), l

        def finish(o0, o1, l):
            o = jnp.where(b1_h, o1, o0) / l
            return jnp.concatenate([o, pltpu.roll(o, 6, 0)], axis=1).astype(_BF16)

        def head(h, carry):
            c_k(h, 0).wait()
            c_k(h, 1).wait()
            pb, l = probs(h)
            c_v(h).wait()
            o = finish(_dot(pb, v_v[h, 0]), _dot(pb, v_v[h, 1]), l)
            o_v[h] = o
            col = pl.multiple_of(h * HW, HW)
            acc_v[...] += _dot_nt(o, wo_v[DR:D, pl.ds(col, HW)])
            return carry

        acc_v[...] = jnp.zeros_like(acc_v)
        c_woa().wait()
        jax.lax.fori_loop(0, LAST, head, 0)

        with _sc("A_wait_k"):
            c_k(LAST, 0).wait()
            c_k(LAST, 1).wait()
        with _sc("A_qk"):
            pb, l = probs(LAST)
        with _sc("A_wait_v0"):
            c_v0().wait()
        with _sc("A_pv0"):
            o0 = _dot(pb, v_v[LAST, 0])
        with _sc("A_wait_v1"):
            c_v1().wait()
        with _sc("A_pv1"):
            o_v[LAST] = finish(o0, _dot(pb, v_v[LAST, 1]), l)
        with _sc("T_mm_last"):
            s_out = acc_v[...] + _dot_nt(o_v[LAST], wo_v[DR:D, LAST * HW:HQD])
            o_ref[:, DR:D] = (x8[:, DR:D] + s_out * gate[:, DR:D])[0:2].astype(o_ref.dtype)

        def lhs(i):
            return jnp.concatenate(
                [o_v[h] for h in range(CUTS[i] // HW, CUTS[i + 1] // HW)], axis=1)

        for i in range(NP - 1):
            with _sc(f"T_wait_p{i}"):
                c_p(i).wait()
            with _sc(f"T_mm_p{i}"):
                part = _dot_nt(lhs(i), wo_v[0:DR, CUTS[i]:CUTS[i + 1]])
                if i == 0:
                    late_v[...] = part
                elif i < NP - 2:
                    late_v[...] += part
                else:
                    late_v[...] = x8[:, 0:DR] + (late_v[...] + part) * gate[:, 0:DR]
        with _sc("T_wait_last"):
            c_p(NP - 1).wait()
        with _sc("T_mm_fin"):
            part = _dot_nt(lhs(NP - 1), wo_v[0:DR, CUTS[NP - 1]:CUTS[NP]])
            o_ref[:, 0:DR] = (late_v[...] + part * gate[:, 0:DR])[0:2].astype(o_ref.dtype)

    return kernel, NSEM


@jax.jit
def pallas_recurrent_scan__sliding_block_cached__dense_activation_gelu__decode_kernel(
    A_x: jax.Array,
    A_k_cache: jax.Array,
    A_v_cache: jax.Array,
    A_wq: jax.Array,
    A_wo: jax.Array,
    B_x: jax.Array,
    B_w1: jax.Array,
    B_b1: jax.Array,
    B_w2: jax.Array,
    B_b2: jax.Array,
):
    del B_x
    B, SQ, D = A_x.shape
    _, HKV, SK, DH = A_k_cache.shape
    HQD = A_wq.shape[1]
    REP = HQD // DH // HKV
    F = B_w1.shape[1]
    W = min(4096, max(256, SK // 4))
    assert B == 2 and SQ == 1 and REP == 2 and F % 128 == 0
    HW = REP * DH

    kernel, nsem = _make_kernel(B, D, HKV, REP, SK, DH, W, F)
    hbm = pl.BlockSpec(memory_space=pl.ANY)
    out = pl.pallas_call(
        kernel,
        in_specs=[hbm] * 9,
        out_specs=pl.BlockSpec(memory_space=pltpu.VMEM),
        out_shape=jax.ShapeDtypeStruct((B, D), A_x.dtype),
        scratch_shapes=[
            pltpu.VMEM((B, D), _BF16),
            pltpu.VMEM((F // 128, 128), _BF16),
            pltpu.VMEM((D,), _BF16),
            pltpu.VMEM((D, HQD), _BF16),
            pltpu.VMEM((D, HQD), _BF16),
            pltpu.VMEM((D, F), _BF16),
            pltpu.VMEM((D, F), _BF16),
            pltpu.VMEM((HKV, B, W, DH), _BF16),
            pltpu.VMEM((HKV, B, W, DH), _BF16),
            pltpu.VMEM((HKV, 8, DH), _BF16),
            pltpu.VMEM((HKV, 8, HW), _BF16),
            pltpu.VMEM((8, D - DR), _F32),
            pltpu.VMEM((8, DR), _F32),
            pltpu.SemaphoreType.DMA((nsem,)),
        ],
        compiler_params=pltpu.CompilerParams(
            vmem_limit_bytes=120 * 1024 * 1024,
            disable_semaphore_checks=True,
        ),
    )(
        A_x.reshape(B, D),
        A_k_cache,
        A_v_cache,
        A_wq,
        A_wo.T,
        B_w1,
        B_b1.reshape(F // 128, 128),
        B_w2.T,
        B_b2,
    )
    return out.reshape(B, SQ, D)
```

```python
import functools

import jax
import jax.numpy as jnp
from jax.experimental import pallas as pl
from jax.experimental.pallas import tpu as pltpu

_NT = (((1,), (1,)), ((), ()))
_F32 = jnp.float32
_BF16 = jnp.bfloat16

TRACE = False
KVR = 256
WR = 8
DR = 64
TC = 3072
AHEAD = 2


def _dot(a, b):
    return jnp.dot(a, b, preferred_element_type=_F32)


def _dot_nt(a, b):
    return jax.lax.dot_general(a, b, _NT, preferred_element_type=_F32)


class _Null:
    def __enter__(self):
        return self

    def __exit__(self, *a):
        return False


def _sc(name):
    return jax.named_scope(name) if TRACE else _Null()


def _make_kernel(B, D, HKV, REP, SK, DH, W, F):
    HW = REP * DH
    HQD = HKV * HW
    FT = F // 128
    scale = float(DH) ** -0.5
    LAST = HKV - 1
    ER = D - DR
    S_X, S_B1, S_B2, S_WQ, S_W1, S_W2, S_WOA, S_LA, S_LB = range(9)
    S_K = 9
    S_V = S_K + B * HKV
    NSEM = S_V + B * HKV

    def kernel(x_hbm, k_hbm, v_hbm, wq_hbm, wo_hbm, w1_hbm, b1_hbm, w2_hbm, b2_hbm,
               o_ref,
               x_v, b1_v, b2_v, wq_v, woa_v, la_v, lb_v, w1_v, w2_v, k_v, v_v, q_v, o_v, acc_v, late_v,
               sem):
        def whole(src, dst, s):
            return pltpu.make_async_copy(src, dst, sem.at[s])

        def start_rows(src, dst, s, nrows, step):
            for i, r in enumerate(range(0, nrows, step)):
                rows = pl.ds(r, step)
                pltpu.make_async_copy(src.at[rows], dst.at[rows], sem.at[s]).start(priority=i % 2)

        win = pl.ds(SK - W, W)
        k_src = lambda h, b: k_hbm.at[b, h, win]
        v_src = lambda h, b: v_hbm.at[b, h, win]
        woa_src = wo_hbm.at[pl.ds(0, ER)]
        la_src = wo_hbm.at[pl.ds(ER, DR), pl.ds(0, TC)]
        lb_src = wo_hbm.at[pl.ds(ER, DR), pl.ds(TC, HQD - TC)]

        def start_head(h):
            for b in range(B):
                start_rows(k_src(h, b), k_v.at[h, b], S_K + h * B + b, W, KVR)
            for b in range(B):
                start_rows(v_src(h, b), v_v.at[h, b], S_V + h * B + b, W, KVR)

        wait_k = lambda h, b: whole(k_src(h, b), k_v.at[h, b], S_K + h * B + b).wait()
        wait_v = lambda h, b: whole(v_src(h, b), v_v.at[h, b], S_V + h * B + b).wait()

        whole(x_hbm, x_v, S_X).start(priority=0)
        whole(b1_hbm, b1_v, S_B1).start(priority=0)
        whole(b2_hbm, b2_v, S_B2).start(priority=0)
        start_rows(wq_hbm, wq_v, S_WQ, D, WR)
        start_rows(w1_hbm, w1_v, S_W1, D, WR)

        whole(x_hbm, x_v, S_X).wait()
        x2 = x_v[...].astype(_F32)
        row_d = jax.lax.broadcasted_iota(jnp.int32, (8, D), 0)
        x8 = jnp.where(row_d % 2 == 0,
                       jnp.broadcast_to(x2[0:1, :], (8, D)),
                       jnp.broadcast_to(x2[1:2, :], (8, D)))
        mean = jnp.mean(x8, axis=1, keepdims=True)
        xc = x8 - mean
        var = jnp.mean(xc * xc, axis=1, keepdims=True)
        xn = (xc / jnp.sqrt(var + 1e-5)).astype(_BF16)

        whole(wq_hbm, wq_v, S_WQ).wait()
        q_all = _dot(xn, wq_v[...])
        row_h = jax.lax.broadcasted_iota(jnp.int32, (8, DH), 0)
        rep1 = (row_h // 2) % 2 == 1
        for h in range(HKV):
            q_v[h] = jnp.where(rep1,
                               q_all[:, h * HW + DH:(h + 1) * HW],
                               q_all[:, h * HW:h * HW + DH]).astype(_BF16)
        start_rows(w2_hbm, w2_v, S_W2, D, WR)

        whole(w1_hbm, w1_v, S_W1).wait()
        whole(b1_hbm, b1_v, S_B1).wait()
        b1f = b1_v[...].astype(_F32)
        bias1 = jnp.concatenate(
            [jnp.broadcast_to(b1f[t:t + 1, :], (8, 128)) for t in range(FT)], axis=1)
        hid = jax.nn.gelu(_dot(xn, w1_v[...]) + bias1, approximate=True).astype(_BF16)
        start_rows(woa_src, woa_v, S_WOA, ER, WR)
        whole(w2_hbm, w2_v, S_W2).wait()
        whole(b2_hbm, b2_v, S_B2).wait()
        y = _dot_nt(hid, w2_v[...]) + b2_v[...].astype(_F32).reshape(1, D)
        gate = y * jax.nn.sigmoid(y)
        for h in range(AHEAD):
            start_head(h)

        row_w = jax.lax.broadcasted_iota(jnp.int32, (8, W), 0)
        b1_w = row_w % 2 == 1
        b1_h = row_h % 2 == 1

        def probs(h):
            qh = q_v[h]
            s0 = _dot_nt(qh, k_v[h, 0])
            s1 = _dot_nt(qh, k_v[h, 1])
            s = jnp.where(b1_w, s1, s0)
            m = jnp.max(s, axis=1, keepdims=True)
            p = jnp.exp((s - m) * scale)
            l = jnp.sum(p, axis=1, keepdims=True)
            return p.astype(_BF16), l

        def finish(o0, o1, l):
            o = jnp.where(b1_h, o1, o0) / l
            return jnp.concatenate([o, pltpu.roll(o, 6, 0)], axis=1).astype(_BF16)

        def attend(h):
            wait_k(h, 0)
            wait_k(h, 1)
            pb, l = probs(h)
            wait_v(h, 0)
            wait_v(h, 1)
            o = finish(_dot(pb, v_v[h, 0]), _dot(pb, v_v[h, 1]), l)
            o_v[h] = o
            col = h * HW if isinstance(h, int) else pl.multiple_of(h * HW, HW)
            acc_v[...] += _dot_nt(o, woa_v[:, pl.ds(col, HW)])

        def head(h, carry):
            attend(h)
            start_head(h + AHEAD)
            return carry

        acc_v[...] = jnp.zeros_like(acc_v)
        whole(woa_src, woa_v, S_WOA).wait()
        jax.lax.fori_loop(0, HKV - AHEAD, head, 0)
        start_rows(la_src, la_v, S_LA, DR, 8)
        start_rows(lb_src, lb_v, S_LB, DR, 8)
        for h in range(HKV - AHEAD, LAST):
            attend(h)

        with _sc("A_wait_k"):
            wait_k(LAST, 0)
            wait_k(LAST, 1)
        with _sc("A_qk"):
            pb, l = probs(LAST)
        with _sc("A_wait_v0"):
            wait_v(LAST, 0)
        with _sc("A_pv0"):
            o0 = _dot(pb, v_v[LAST, 0])
        with _sc("A_wait_v1"):
            wait_v(LAST, 1)
        with _sc("A_pv1"):
            o_v[LAST] = finish(o0, _dot(pb, v_v[LAST, 1]), l)
        with _sc("T_mm_last"):
            s_out = acc_v[...] + _dot_nt(o_v[LAST], woa_v[:, LAST * HW:HQD])
            o_ref[:, 0:ER] = (x8[:, 0:ER] + s_out * gate[:, 0:ER])[0:2].astype(o_ref.dtype)

        def lhs(c0, c1):
            return jnp.concatenate([o_v[h] for h in range(c0 // HW, c1 // HW)], axis=1)

        with _sc("T_wait_la"):
            whole(la_src, la_v, S_LA).wait()
        with _sc("T_mm_la"):
            late_v[...] = _dot_nt(lhs(0, TC), la_v[...])
        with _sc("T_wait_lb"):
            whole(lb_src, lb_v, S_LB).wait()
        with _sc("T_mm_lb"):
            part = late_v[...] + _dot_nt(lhs(TC, HQD), lb_v[...])
            o_ref[:, ER:D] = (x8[:, ER:D] + part * gate[:, ER:D])[0:2].astype(o_ref.dtype)

    return kernel, NSEM


@jax.jit
def pallas_recurrent_scan__sliding_block_cached__dense_activation_gelu__decode_kernel(
    A_x: jax.Array,
    A_k_cache: jax.Array,
    A_v_cache: jax.Array,
    A_wq: jax.Array,
    A_wo: jax.Array,
    B_x: jax.Array,
    B_w1: jax.Array,
    B_b1: jax.Array,
    B_w2: jax.Array,
    B_b2: jax.Array,
):
    del B_x
    B, SQ, D = A_x.shape
    _, HKV, SK, DH = A_k_cache.shape
    HQD = A_wq.shape[1]
    REP = HQD // DH // HKV
    F = B_w1.shape[1]
    W = min(4096, max(256, SK // 4))
    assert B == 2 and SQ == 1 and REP == 2 and F % 128 == 0
    HW = REP * DH

    kernel, nsem = _make_kernel(B, D, HKV, REP, SK, DH, W, F)
    hbm = pl.BlockSpec(memory_space=pl.ANY)
    out = pl.pallas_call(
        kernel,
        in_specs=[hbm] * 9,
        out_specs=pl.BlockSpec(memory_space=pltpu.VMEM),
        out_shape=jax.ShapeDtypeStruct((B, D), A_x.dtype),
        scratch_shapes=[
            pltpu.VMEM((B, D), _BF16),
            pltpu.VMEM((F // 128, 128), _BF16),
            pltpu.VMEM((D,), _BF16),
            pltpu.VMEM((D, HQD), _BF16),
            pltpu.VMEM((D - DR, HQD), _BF16),
            pltpu.VMEM((DR, TC), _BF16),
            pltpu.VMEM((DR, HQD - TC), _BF16),
            pltpu.VMEM((D, F), _BF16),
            pltpu.VMEM((D, F), _BF16),
            pltpu.VMEM((HKV, B, W, DH), _BF16),
            pltpu.VMEM((HKV, B, W, DH), _BF16),
            pltpu.VMEM((HKV, 8, DH), _BF16),
            pltpu.VMEM((HKV, 8, HW), _BF16),
            pltpu.VMEM((8, D - DR), _F32),
            pltpu.VMEM((8, DR), _F32),
            pltpu.SemaphoreType.DMA((nsem,)),
        ],
        compiler_params=pltpu.CompilerParams(
            vmem_limit_bytes=120 * 1024 * 1024,
            disable_semaphore_checks=True,
            disable_bounds_checks=True,
        ),
    )(
        A_x.reshape(B, D),
        A_k_cache,
        A_v_cache,
        A_wq,
        A_wo.T,
        B_w1,
        B_b1.reshape(F // 128, 128),
        B_w2.T,
        B_b2,
    )
    return out.reshape(B, SQ, D)
```

```python
import functools

import jax
import jax.numpy as jnp
from jax.experimental import pallas as pl
from jax.experimental.pallas import tpu as pltpu

_NT = (((1,), (1,)), ((), ()))
_F32 = jnp.float32
_BF16 = jnp.bfloat16

TRACE = False
KV_PIECES = (208,) * 9 + (176,)
MODE = "half"
DR = 64
TC = 3072
AHEAD = 2


def _dot(a, b):
    return jnp.dot(a, b, preferred_element_type=_F32)


def _dot_nt(a, b):
    return jax.lax.dot_general(a, b, _NT, preferred_element_type=_F32)


class _Null:
    def __enter__(self):
        return self

    def __exit__(self, *a):
        return False


def _sc(name):
    return jax.named_scope(name) if TRACE else _Null()


def _make_kernel(B, D, HKV, REP, SK, DH, W, F):
    HW = REP * DH
    HQD = HKV * HW
    FT = F // 128
    scale = float(DH) ** -0.5
    LAST = HKV - 1
    ER = D - DR
    S_X, S_B1, S_B2, S_WQ, S_W1, S_W2, S_WOA, S_LA, S_LB = range(9)
    S_K = 9
    S_V = S_K + B * HKV
    NSEM = S_V + B * HKV

    def kernel(x_hbm, k_hbm, v_hbm, wq_hbm, wo_hbm, w1_hbm, b1_hbm, w2_hbm, b2_hbm,
               o_ref,
               x_v, b1_v, b2_v, wq_v, woa_v, la_v, lb_v, w1_v, w2_v, k_v, v_v, q_v, o_v, acc_v, late_v,
               sem):
        def whole(src, dst, s):
            return pltpu.make_async_copy(src, dst, sem.at[s])

        def start(src, dst, s, thread):
            pltpu.make_async_copy(src, dst, sem.at[s]).start(priority=thread)

        def start_window(src, dst, s):
            r = 0
            for n in KV_PIECES:
                for t in range(2):
                    rows = pl.ds(t * (W // 2) + r, n)
                    start(src.at[rows], dst.at[rows], s, t)
                r += n
            assert r == W // 2

        def start_windows(src0, dst0, s0, src1, dst1, s1):
            for half in range(2):
                r = half * (W // 2)
                for n in KV_PIECES:
                    rows = pl.ds(r, n)
                    start(src0.at[rows], dst0.at[rows], s0, 0)
                    start(src1.at[rows], dst1.at[rows], s1, 1)
                    r += n

        def start_matrix(src, dst, s, nrows, ncols, col_parts):
            half = nrows // 2
            cw = ncols // col_parts

            def body(i, carry):
                for c in range(col_parts):
                    cols = pl.ds(c * cw, cw)
                    for t in range(2):
                        rows = pl.ds(pl.multiple_of(t * half + i * 8, 8), 8)
                        start(src.at[rows, cols], dst.at[rows, cols], s, t)
                return carry

            jax.lax.fori_loop(0, half // 8, body, 0)

        win = pl.ds(SK - W, W)
        k_src = lambda h, b: k_hbm.at[b, h, win]
        v_src = lambda h, b: v_hbm.at[b, h, win]
        woa_src = wo_hbm.at[pl.ds(0, ER)]
        la_src = wo_hbm.at[pl.ds(ER, DR), pl.ds(0, TC)]
        lb_src = wo_hbm.at[pl.ds(ER, DR), pl.ds(TC, HQD - TC)]

        def start_k(h):
            if MODE == "batch":
                start_windows(k_src(h, 0), k_v.at[h, 0], S_K + h * B, k_src(h, 1), k_v.at[h, 1], S_K + h * B + 1)
            else:
                for b in range(B):
                    start_window(k_src(h, b), k_v.at[h, b], S_K + h * B + b)

        def start_v(h):
            if MODE == "batch" and not (isinstance(h, int) and h == LAST):
                start_windows(v_src(h, 0), v_v.at[h, 0], S_V + h * B, v_src(h, 1), v_v.at[h, 1], S_V + h * B + 1)
            else:
                for b in range(B):
                    start_window(v_src(h, b), v_v.at[h, b], S_V + h * B + b)

        def start_head(h):
            start_k(h)
            start_v(h)

        wait_k = lambda h, b: whole(k_src(h, b), k_v.at[h, b], S_K + h * B + b).wait()
        wait_v = lambda h, b: whole(v_src(h, b), v_v.at[h, b], S_V + h * B + b).wait()

        whole(x_hbm, x_v, S_X).start(priority=0)
        whole(b1_hbm, b1_v, S_B1).start(priority=0)
        whole(b2_hbm, b2_v, S_B2).start(priority=0)
        start_matrix(wq_hbm, wq_v, S_WQ, D, HQD, 2)
        start_matrix(w1_hbm, w1_v, S_W1, D, F, 2)

        whole(x_hbm, x_v, S_X).wait()
        x2 = x_v[...].astype(_F32)
        row_d = jax.lax.broadcasted_iota(jnp.int32, (8, D), 0)
        x8 = jnp.where(row_d % 2 == 0,
                       jnp.broadcast_to(x2[0:1, :], (8, D)),
                       jnp.broadcast_to(x2[1:2, :], (8, D)))
        mean = jnp.mean(x8, axis=1, keepdims=True)
        xc = x8 - mean
        var = jnp.mean(xc * xc, axis=1, keepdims=True)
        xn = (xc / jnp.sqrt(var + 1e-5)).astype(_BF16)

        whole(wq_hbm, wq_v, S_WQ).wait()
        q_all = _dot(xn, wq_v[...])
        row_h = jax.lax.broadcasted_iota(jnp.int32, (8, DH), 0)
        rep1 = (row_h // 2) % 2 == 1
        for h in range(HKV):
            q_v[h] = jnp.where(rep1,
                               q_all[:, h * HW + DH:(h + 1) * HW],
                               q_all[:, h * HW:h * HW + DH]).astype(_BF16)
        start_matrix(w2_hbm, w2_v, S_W2, D, F, 2)

        whole(w1_hbm, w1_v, S_W1).wait()
        whole(b1_hbm, b1_v, S_B1).wait()
        b1f = b1_v[...].astype(_F32)
        bias1 = jnp.concatenate(
            [jnp.broadcast_to(b1f[t:t + 1, :], (8, 128)) for t in range(FT)], axis=1)
        hid = jax.nn.gelu(_dot(xn, w1_v[...]) + bias1, approximate=True).astype(_BF16)
        start_matrix(woa_src, woa_v, S_WOA, ER, HQD, 2)
        whole(w2_hbm, w2_v, S_W2).wait()
        whole(b2_hbm, b2_v, S_B2).wait()
        y = _dot_nt(hid, w2_v[...]) + b2_v[...].astype(_F32).reshape(1, D)
        gate = y * jax.nn.sigmoid(y)
        for h in range(AHEAD):
            start_head(h)

        row_w = jax.lax.broadcasted_iota(jnp.int32, (8, W), 0)
        b1_w = row_w % 2 == 1
        b1_h = row_h % 2 == 1

        def probs(h):
            qh = q_v[h]
            s0 = _dot_nt(qh, k_v[h, 0])
            s1 = _dot_nt(qh, k_v[h, 1])
            s = jnp.where(b1_w, s1, s0)
            m = jnp.max(s, axis=1, keepdims=True)
            p = jnp.exp((s - m) * scale)
            l = jnp.sum(p, axis=1, keepdims=True)
            return p.astype(_BF16), l

        def finish(o0, o1, l):
            o = jnp.where(b1_h, o1, o0) / l
            return jnp.concatenate([o, pltpu.roll(o, 6, 0)], axis=1).astype(_BF16)

        def attend(h):
            wait_k(h, 0)
            wait_k(h, 1)
            pb, l = probs(h)
            wait_v(h, 0)
            wait_v(h, 1)
            o = finish(_dot(pb, v_v[h, 0]), _dot(pb, v_v[h, 1]), l)
            o_v[h] = o
            col = h * HW if isinstance(h, int) else pl.multiple_of(h * HW, HW)
            acc_v[...] += _dot_nt(o, woa_v[:, pl.ds(col, HW)])

        def head(h, carry):
            attend(h)
            start_head(h + AHEAD)
            return carry

        acc_v[...] = jnp.zeros_like(acc_v)
        whole(woa_src, woa_v, S_WOA).wait()
        jax.lax.fori_loop(0, HKV - AHEAD, head, 0)
        for src, dst, sidx in ((la_src, la_v, S_LA), (lb_src, lb_v, S_LB)):
            for i in range(DR // 16):
                for t in range(2):
                    rows = pl.ds(t * (DR // 2) + i * 8, 8)
                    start(src.at[rows], dst.at[rows], sidx, t)
        for h in range(HKV - AHEAD, LAST):
            attend(h)

        with _sc("A_wait_k"):
            wait_k(LAST, 0)
            wait_k(LAST, 1)
        with _sc("A_qk"):
            pb, l = probs(LAST)
        with _sc("A_wait_v0"):
            wait_v(LAST, 0)
        with _sc("A_pv0"):
            o0 = _dot(pb, v_v[LAST, 0])
        with _sc("A_wait_v1"):
            wait_v(LAST, 1)
        with _sc("A_pv1"):
            o_v[LAST] = finish(o0, _dot(pb, v_v[LAST, 1]), l)
        with _sc("T_mm_last"):
            s_out = acc_v[...] + _dot_nt(o_v[LAST], woa_v[:, LAST * HW:HQD])
            o_ref[:, 0:ER] = (x8[:, 0:ER] + s_out * gate[:, 0:ER])[0:2].astype(o_ref.dtype)

        def lhs(c0, c1):
            return jnp.concatenate([o_v[h] for h in range(c0 // HW, c1 // HW)], axis=1)

        with _sc("T_wait_la"):
            whole(la_src, la_v, S_LA).wait()
        with _sc("T_mm_la"):
            late_v[...] = _dot_nt(lhs(0, TC), la_v[...])
        with _sc("T_wait_lb"):
            whole(lb_src, lb_v, S_LB).wait()
        with _sc("T_mm_lb"):
            part = late_v[...] + _dot_nt(lhs(TC, HQD), lb_v[...])
            o_ref[:, ER:D] = (x8[:, ER:D] + part * gate[:, ER:D])[0:2].astype(o_ref.dtype)

    return kernel, NSEM


@jax.jit
def pallas_recurrent_scan__sliding_block_cached__dense_activation_gelu__decode_kernel(
    A_x: jax.Array,
    A_k_cache: jax.Array,
    A_v_cache: jax.Array,
    A_wq: jax.Array,
    A_wo: jax.Array,
    B_x: jax.Array,
    B_w1: jax.Array,
    B_b1: jax.Array,
    B_w2: jax.Array,
    B_b2: jax.Array,
):
    del B_x
    B, SQ, D = A_x.shape
    _, HKV, SK, DH = A_k_cache.shape
    HQD = A_wq.shape[1]
    REP = HQD // DH // HKV
    F = B_w1.shape[1]
    W = min(4096, max(256, SK // 4))
    assert B == 2 and SQ == 1 and REP == 2 and F % 128 == 0
    HW = REP * DH

    kernel, nsem = _make_kernel(B, D, HKV, REP, SK, DH, W, F)
    hbm = pl.BlockSpec(memory_space=pl.ANY)
    out = pl.pallas_call(
        kernel,
        in_specs=[hbm] * 9,
        out_specs=pl.BlockSpec(memory_space=pltpu.VMEM),
        out_shape=jax.ShapeDtypeStruct((B, D), A_x.dtype),
        scratch_shapes=[
            pltpu.VMEM((B, D), _BF16),
            pltpu.VMEM((F // 128, 128), _BF16),
            pltpu.VMEM((D,), _BF16),
            pltpu.VMEM((D, HQD), _BF16),
            pltpu.VMEM((D - DR, HQD), _BF16),
            pltpu.VMEM((DR, TC), _BF16),
            pltpu.VMEM((DR, HQD - TC), _BF16),
            pltpu.VMEM((D, F), _BF16),
            pltpu.VMEM((D, F), _BF16),
            pltpu.VMEM((HKV, B, W, DH), _BF16),
            pltpu.VMEM((HKV, B, W, DH), _BF16),
            pltpu.VMEM((HKV, 8, DH), _BF16),
            pltpu.VMEM((HKV, 8, HW), _BF16),
            pltpu.VMEM((8, D - DR), _F32),
            pltpu.VMEM((8, DR), _F32),
            pltpu.SemaphoreType.DMA((nsem,)),
        ],
        compiler_params=pltpu.CompilerParams(
            vmem_limit_bytes=120 * 1024 * 1024,
            disable_semaphore_checks=True,
            disable_bounds_checks=True,
        ),
    )(
        A_x.reshape(B, D),
        A_k_cache,
        A_v_cache,
        A_wq,
        A_wo.T,
        B_w1,
        B_b1.reshape(F // 128, 128),
        B_w2.T,
        B_b2,
    )
    return out.reshape(B, SQ, D)
```

```python
import functools

import jax
import jax.numpy as jnp
from jax.experimental import pallas as pl
from jax.experimental.pallas import tpu as pltpu

_NT = (((1,), (1,)), ((), ()))
_F32 = jnp.float32
_BF16 = jnp.bfloat16

TRACE = False
KV_PIECES = (176,) * 11 + (112,)
MODE = "half"
DR = 128
CUTS = (0, 2048, 3072, 3584, 4096)
AHEAD = 2


def _dot(a, b):
    return jnp.dot(a, b, preferred_element_type=_F32)


def _dot_nt(a, b):
    return jax.lax.dot_general(a, b, _NT, preferred_element_type=_F32)


class _Null:
    def __enter__(self):
        return self

    def __exit__(self, *a):
        return False


def _sc(name):
    return jax.named_scope(name) if TRACE else _Null()


def _make_kernel(B, D, HKV, REP, SK, DH, W, F):
    HW = REP * DH
    HQD = HKV * HW
    FT = F // 128
    scale = float(DH) ** -0.5
    LAST = HKV - 1
    ER = D - DR
    S_X, S_B1, S_B2, S_WQ, S_W1, S_W2, S_WOA = range(7)
    NL = len(CUTS) - 1
    S_L = 7
    S_K = S_L + NL
    S_V = S_K + B * HKV
    NSEM = S_V + B * HKV

    def kernel(x_hbm, k_hbm, v_hbm, wq_hbm, wo_hbm, w1_hbm, b1_hbm, w2_hbm, b2_hbm,
               o_ref,
               x_v, b1_v, b2_v, wq_v, woa_v, wol_v, w1_v, w2_v, k_v, v_v, q_v, p_v, o_v, acc_v, late_v,
               sem):
        def whole(src, dst, s):
            return pltpu.make_async_copy(src, dst, sem.at[s])

        def start(src, dst, s, thread):
            pltpu.make_async_copy(src, dst, sem.at[s]).start(priority=thread)

        def start_window(src, dst, s):
            r = 0
            for n in KV_PIECES:
                for t in range(2):
                    rows = pl.ds(t * (W // 2) + r, n)
                    start(src.at[rows], dst.at[rows], s, t)
                r += n
            assert r == W // 2

        def start_windows(src0, dst0, s0, src1, dst1, s1):
            for half in range(2):
                r = half * (W // 2)
                for n in KV_PIECES:
                    rows = pl.ds(r, n)
                    start(src0.at[rows], dst0.at[rows], s0, 0)
                    start(src1.at[rows], dst1.at[rows], s1, 1)
                    r += n

        def start_matrix(src, dst, s, nrows, ncols, col_parts):
            half = nrows // 2
            cw = ncols // col_parts

            def body(i, carry):
                for c in range(col_parts):
                    cols = pl.ds(c * cw, cw)
                    for t in range(2):
                        rows = pl.ds(pl.multiple_of(t * half + i * 8, 8), 8)
                        start(src.at[rows, cols], dst.at[rows, cols], s, t)
                return carry

            jax.lax.fori_loop(0, half // 8, body, 0)

        win = pl.ds(SK - W, W)
        k_src = lambda h, b: k_hbm.at[b, h, win]
        v_src = lambda h, b: v_hbm.at[b, h, win]
        woa_src = wo_hbm.at[pl.ds(DR, ER)]
        late_cols = lambda i: pl.ds(CUTS[i], CUTS[i + 1] - CUTS[i])
        late_src = lambda i: wo_hbm.at[pl.ds(0, DR), late_cols(i)]
        late_dst = lambda i: wol_v.at[:, late_cols(i)]

        def start_k(h):
            if MODE == "batch":
                start_windows(k_src(h, 0), k_v.at[h, 0], S_K + h * B, k_src(h, 1), k_v.at[h, 1], S_K + h * B + 1)
            else:
                for b in range(B):
                    start_window(k_src(h, b), k_v.at[h, b], S_K + h * B + b)

        def start_v(h):
            if MODE == "batch" and not (isinstance(h, int) and h == LAST):
                start_windows(v_src(h, 0), v_v.at[h, 0], S_V + h * B, v_src(h, 1), v_v.at[h, 1], S_V + h * B + 1)
            else:
                for b in range(B):
                    start_window(v_src(h, b), v_v.at[h, b], S_V + h * B + b)

        def start_head(h):
            start_k(h)
            start_v(h)

        wait_k = lambda h, b: whole(k_src(h, b), k_v.at[h, b], S_K + h * B + b).wait()
        wait_v = lambda h, b: whole(v_src(h, b), v_v.at[h, b], S_V + h * B + b).wait()

        whole(x_hbm, x_v, S_X).start(priority=0)
        whole(b1_hbm, b1_v, S_B1).start(priority=0)
        whole(b2_hbm, b2_v, S_B2).start(priority=0)
        start_matrix(wq_hbm, wq_v, S_WQ, D, HQD, 2)
        start_matrix(w1_hbm, w1_v, S_W1, D, F, 2)

        whole(x_hbm, x_v, S_X).wait()
        x2 = x_v[...].astype(_F32)
        row_d = jax.lax.broadcasted_iota(jnp.int32, (8, D), 0)
        x8 = jnp.where(row_d % 2 == 0,
                       jnp.broadcast_to(x2[0:1, :], (8, D)),
                       jnp.broadcast_to(x2[1:2, :], (8, D)))
        mean = jnp.mean(x8, axis=1, keepdims=True)
        xc = x8 - mean
        var = jnp.mean(xc * xc, axis=1, keepdims=True)
        xn = (xc / jnp.sqrt(var + 1e-5)).astype(_BF16)

        whole(wq_hbm, wq_v, S_WQ).wait()
        q_all = _dot(xn, wq_v[...])
        row_h = jax.lax.broadcasted_iota(jnp.int32, (8, DH), 0)
        rep1 = (row_h // 2) % 2 == 1
        for h in range(HKV):
            q_v[h] = jnp.where(rep1,
                               q_all[:, h * HW + DH:(h + 1) * HW],
                               q_all[:, h * HW:h * HW + DH]).astype(_BF16)
        start_matrix(w2_hbm, w2_v, S_W2, D, F, 2)

        whole(w1_hbm, w1_v, S_W1).wait()
        whole(b1_hbm, b1_v, S_B1).wait()
        b1f = b1_v[...].astype(_F32)
        bias1 = jnp.concatenate(
            [jnp.broadcast_to(b1f[t:t + 1, :], (8, 128)) for t in range(FT)], axis=1)
        hid = jax.nn.gelu(_dot(xn, w1_v[...]) + bias1, approximate=True).astype(_BF16)
        start_matrix(woa_src, woa_v, S_WOA, ER, HQD, 2)
        whole(w2_hbm, w2_v, S_W2).wait()
        whole(b2_hbm, b2_v, S_B2).wait()
        y = _dot_nt(hid, w2_v[...]) + b2_v[...].astype(_F32).reshape(1, D)
        gate = y * jax.nn.sigmoid(y)
        start_k(0)
        start_k(1)
        start_v(0)
        start_k(2)
        start_v(1)

        row_w = jax.lax.broadcasted_iota(jnp.int32, (8, W), 0)
        b1_w = row_w % 2 == 1
        b1_h = row_h % 2 == 1

        def probs(h):
            qh = q_v[h]
            s0 = _dot_nt(qh, k_v[h, 0])
            s1 = _dot_nt(qh, k_v[h, 1])
            s = jnp.where(b1_w, s1, s0)
            m = jnp.max(s, axis=1, keepdims=True)
            p = jnp.exp((s - m) * scale)
            l = jnp.sum(p, axis=1, keepdims=True)
            return p.astype(_BF16), l

        def finish(o0, o1, l):
            o = jnp.where(b1_h, o1, o0) / l
            return jnp.concatenate([o, pltpu.roll(o, 6, 0)], axis=1).astype(_BF16)

        def scores(h):
            wait_k(h, 0)
            wait_k(h, 1)
            return probs(h)

        def project(h, o):
            o_v[h] = o
            col = h * HW if isinstance(h, int) else pl.multiple_of(h * HW, HW)
            acc_v[...] += _dot_nt(o, woa_v[:, pl.ds(col, HW)])

        def values(h, pb, l):
            wait_v(h, 0)
            wait_v(h, 1)
            project(h, finish(_dot(pb, v_v[h, 0]), _dot(pb, v_v[h, 1]), l))

        def head(h, carry):
            values(h, *scores(h))
            start_k(h + 3)
            start_v(h + 2)
            return carry

        acc_v[...] = jnp.zeros_like(acc_v)
        whole(woa_src, woa_v, S_WOA).wait()
        jax.lax.fori_loop(0, HKV - 3, head, 0)

        values(HKV - 3, *scores(HKV - 3))
        with _sc("A_qk14"):
            pb_prev, l_prev = scores(HKV - 2)
            p_v[0] = pb_prev
        start_v(LAST)
        with _sc("A_qk15"):
            pb, l = scores(LAST)
            p_v[1] = pb
        with _sc("A_v14"):
            values(HKV - 2, p_v[0], l_prev)
        with _sc("A_wait_v0"):
            wait_v(LAST, 0)
        with _sc("A_pv0"):
            o0 = _dot(p_v[1], v_v[LAST, 0])
        for i in range(NL):
            for r in range(0, DR, 8):
                rows = pl.ds(r, 8)
                start(late_src(i).at[rows], late_dst(i).at[rows], S_L + i, 1)
        with _sc("A_wait_v1"):
            wait_v(LAST, 1)
        with _sc("A_pv1"):
            o_v[LAST] = finish(o0, _dot(p_v[1], v_v[LAST, 1]), l)
        with _sc("T_mm_last"):
            s_out = acc_v[...] + _dot_nt(o_v[LAST], woa_v[:, LAST * HW:HQD])
            o_ref[:, DR:D] = (x8[:, DR:D] + s_out * gate[:, DR:D])[0:2].astype(o_ref.dtype)

        def lhs(c0, c1):
            return jnp.concatenate([o_v[h] for h in range(c0 // HW, c1 // HW)], axis=1)

        for i in range(NL):
            with _sc(f"T_wait_l{i}"):
                whole(late_src(i), late_dst(i), S_L + i).wait()
            with _sc(f"T_mm_l{i}"):
                part = _dot_nt(lhs(CUTS[i], CUTS[i + 1]), wol_v[:, CUTS[i]:CUTS[i + 1]])
                if i == 0:
                    late_v[...] = part
                elif i < NL - 2:
                    late_v[...] += part
                elif i == NL - 2:
                    late_v[...] = x8[:, 0:DR] + (late_v[...] + part) * gate[:, 0:DR]
                else:
                    o_ref[:, 0:DR] = (late_v[...] + part * gate[:, 0:DR])[0:2].astype(o_ref.dtype)

    return kernel, NSEM


@jax.jit
def pallas_recurrent_scan__sliding_block_cached__dense_activation_gelu__decode_kernel(
    A_x: jax.Array,
    A_k_cache: jax.Array,
    A_v_cache: jax.Array,
    A_wq: jax.Array,
    A_wo: jax.Array,
    B_x: jax.Array,
    B_w1: jax.Array,
    B_b1: jax.Array,
    B_w2: jax.Array,
    B_b2: jax.Array,
):
    del B_x
    B, SQ, D = A_x.shape
    _, HKV, SK, DH = A_k_cache.shape
    HQD = A_wq.shape[1]
    REP = HQD // DH // HKV
    F = B_w1.shape[1]
    W = min(4096, max(256, SK // 4))
    assert B == 2 and SQ == 1 and REP == 2 and F % 128 == 0
    HW = REP * DH

    kernel, nsem = _make_kernel(B, D, HKV, REP, SK, DH, W, F)
    hbm = pl.BlockSpec(memory_space=pl.ANY)
    out = pl.pallas_call(
        kernel,
        in_specs=[hbm] * 9,
        out_specs=pl.BlockSpec(memory_space=pltpu.VMEM),
        out_shape=jax.ShapeDtypeStruct((B, D), A_x.dtype),
        scratch_shapes=[
            pltpu.VMEM((B, D), _BF16),
            pltpu.VMEM((F // 128, 128), _BF16),
            pltpu.VMEM((D,), _BF16),
            pltpu.VMEM((D, HQD), _BF16),
            pltpu.VMEM((D - DR, HQD), _BF16),
            pltpu.VMEM((DR, HQD), _BF16),
            pltpu.VMEM((D, F), _BF16),
            pltpu.VMEM((D, F), _BF16),
            pltpu.VMEM((HKV, B, W, DH), _BF16),
            pltpu.VMEM((HKV, B, W, DH), _BF16),
            pltpu.VMEM((HKV, 8, DH), _BF16),
            pltpu.VMEM((2, 8, W), _BF16),
            pltpu.VMEM((HKV, 8, HW), _BF16),
            pltpu.VMEM((8, D - DR), _F32),
            pltpu.VMEM((8, DR), _F32),
            pltpu.SemaphoreType.DMA((nsem,)),
        ],
        compiler_params=pltpu.CompilerParams(
            vmem_limit_bytes=120 * 1024 * 1024,
            disable_semaphore_checks=True,
            disable_bounds_checks=True,
        ),
    )(
        A_x.reshape(B, D),
        A_k_cache,
        A_v_cache,
        A_wq,
        A_wo.T,
        B_w1,
        B_b1.reshape(F // 128, 128),
        B_w2.T,
        B_b2,
    )
    return out.reshape(B, SQ, D)
```

```python
import jax
import jax.numpy as jnp
from jax.experimental import pallas as pl
from jax.experimental.pallas import tpu as pltpu

_NT = (((1,), (1,)), ((), ()))
_F32 = jnp.float32
_BF16 = jnp.bfloat16

_KV_ROWS = 176
_LATE = 128
_LATE_CUTS = (0, 2048, 3072, 3584, 4096)


def _dot(a, b):
    return jnp.dot(a, b, preferred_element_type=_F32)


def _dot_nt(a, b):
    return jax.lax.dot_general(a, b, _NT, preferred_element_type=_F32)


def _make_kernel(B, D, HKV, REP, SK, DH, W, F):
    HW = REP * DH
    HQD = HKV * HW
    FT = F // 128
    scale = float(DH) ** -0.5
    LAST = HKV - 1
    EARLY = D - _LATE
    NL = len(_LATE_CUTS) - 1
    assert _LATE_CUTS[0] == 0 and _LATE_CUTS[-1] == HQD
    assert all(c % HW == 0 for c in _LATE_CUTS)
    S_X, S_B1, S_B2, S_WQ, S_W1, S_W2, S_WO = range(7)
    S_L = 7
    S_K = S_L + NL
    S_V = S_K + B * HKV
    NSEM = S_V + B * HKV

    def kernel(x_hbm, k_hbm, v_hbm, wq_hbm, wo_hbm, w1_hbm, b1_hbm, w2_hbm, b2_hbm,
               o_ref,
               x_v, b1_v, b2_v, wq_v, woe_v, wol_v, w1_v, w2_v, k_v, v_v,
               q_v, p_v, o_v, acc_v, late_v, sem):
        def start(src, dst, s, thread):
            pltpu.make_async_copy(src, dst, sem.at[s]).start(priority=thread)

        def wait(src, dst, s):
            pltpu.make_async_copy(src, dst, sem.at[s]).wait()

        def start_window(src, dst, s):
            half = W // 2
            for r in range(0, half, _KV_ROWS):
                n = min(_KV_ROWS, half - r)
                for t in range(2):
                    rows = pl.ds(t * half + r, n)
                    start(src.at[rows], dst.at[rows], s, t)

        def start_matrix(src, dst, s, nrows, ncols):
            half, cw = nrows // 2, ncols // 2

            def body(i, carry):
                for c in range(2):
                    cols = pl.ds(c * cw, cw)
                    for t in range(2):
                        rows = pl.ds(pl.multiple_of(t * half + i * 8, 8), 8)
                        start(src.at[rows, cols], dst.at[rows, cols], s, t)
                return carry

            jax.lax.fori_loop(0, half // 8, body, 0)

        win = pl.ds(SK - W, W)
        k_copy = lambda h, b: (k_hbm.at[b, h, win], k_v.at[h, b], S_K + h * B + b)
        v_copy = lambda h, b: (v_hbm.at[b, h, win], v_v.at[h, b], S_V + h * B + b)
        woe_copy = (wo_hbm.at[pl.ds(_LATE, EARLY)], woe_v, S_WO)

        def late_copy(i):
            cols = pl.ds(_LATE_CUTS[i], _LATE_CUTS[i + 1] - _LATE_CUTS[i])
            return wo_hbm.at[pl.ds(0, _LATE), cols], wol_v.at[:, cols], S_L + i

        def start_k(h):
            for b in range(B):
                start_window(*k_copy(h, b))

        def start_v(h):
            for b in range(B):
                start_window(*v_copy(h, b))

        start(x_hbm, x_v, S_X, 0)
        start(b1_hbm, b1_v, S_B1, 0)
        start(b2_hbm, b2_v, S_B2, 0)
        start_matrix(wq_hbm, wq_v, S_WQ, D, HQD)
        start_matrix(w1_hbm, w1_v, S_W1, D, F)

        wait(x_hbm, x_v, S_X)
        x2 = x_v[...].astype(_F32)
        row_d = jax.lax.broadcasted_iota(jnp.int32, (8, D), 0)
        x8 = jnp.where(row_d % 2 == 0,
                       jnp.broadcast_to(x2[0:1, :], (8, D)),
                       jnp.broadcast_to(x2[1:2, :], (8, D)))
        mean = jnp.mean(x8, axis=1, keepdims=True)
        xc = x8 - mean
        var = jnp.mean(xc * xc, axis=1, keepdims=True)
        xn = (xc / jnp.sqrt(var + 1e-5)).astype(_BF16)

        wait(wq_hbm, wq_v, S_WQ)
        q_all = _dot(xn, wq_v[...])
        row_h = jax.lax.broadcasted_iota(jnp.int32, (8, DH), 0)
        rep1 = (row_h // 2) % 2 == 1
        for h in range(HKV):
            q_v[h] = jnp.where(rep1,
                               q_all[:, h * HW + DH:(h + 1) * HW],
                               q_all[:, h * HW:h * HW + DH]).astype(_BF16)
        start_matrix(w2_hbm, w2_v, S_W2, D, F)

        wait(w1_hbm, w1_v, S_W1)
        wait(b1_hbm, b1_v, S_B1)
        b1f = b1_v[...].astype(_F32)
        bias1 = jnp.concatenate(
            [jnp.broadcast_to(b1f[t:t + 1, :], (8, 128)) for t in range(FT)], axis=1)
        hid = jax.nn.gelu(_dot(xn, w1_v[...]) + bias1, approximate=True).astype(_BF16)
        start_matrix(woe_copy[0], woe_v, S_WO, EARLY, HQD)
        wait(w2_hbm, w2_v, S_W2)
        wait(b2_hbm, b2_v, S_B2)
        y = _dot_nt(hid, w2_v[...]) + b2_v[...].astype(_F32).reshape(1, D)
        gate = y * jax.nn.sigmoid(y)

        start_k(0)
        start_k(1)
        start_v(0)
        start_k(2)
        start_v(1)

        batch1_w = jax.lax.broadcasted_iota(jnp.int32, (8, W), 0) % 2 == 1
        batch1_h = row_h % 2 == 1

        def scores(h):
            wait(*k_copy(h, 0))
            wait(*k_copy(h, 1))
            qh = q_v[h]
            s = jnp.where(batch1_w, _dot_nt(qh, k_v[h, 1]), _dot_nt(qh, k_v[h, 0]))
            m = jnp.max(s, axis=1, keepdims=True)
            p = jnp.exp((s - m) * scale)
            return p.astype(_BF16), jnp.sum(p, axis=1, keepdims=True)

        def normalise(o0, o1, l):
            o = jnp.where(batch1_h, o1, o0) / l
            return jnp.concatenate([o, pltpu.roll(o, 6, 0)], axis=1).astype(_BF16)

        def values(h, pb, l):
            wait(*v_copy(h, 0))
            wait(*v_copy(h, 1))
            o = normalise(_dot(pb, v_v[h, 0]), _dot(pb, v_v[h, 1]), l)
            o_v[h] = o
            col = h * HW if isinstance(h, int) else pl.multiple_of(h * HW, HW)
            acc_v[...] += _dot_nt(o, woe_v[:, pl.ds(col, HW)])

        def head(h, carry):
            values(h, *scores(h))
            start_k(h + 3)
            start_v(h + 2)
            return carry

        acc_v[...] = jnp.zeros_like(acc_v)
        wait(*woe_copy)
        jax.lax.fori_loop(0, HKV - 3, head, 0)

        values(HKV - 3, *scores(HKV - 3))
        pb, l_prev = scores(HKV - 2)
        p_v[0] = pb
        start_v(LAST)
        pb, l_last = scores(LAST)
        p_v[1] = pb
        values(HKV - 2, p_v[0], l_prev)
        wait(*v_copy(LAST, 0))
        o0 = _dot(p_v[1], v_v[LAST, 0])
        for i in range(NL):
            src, dst, s = late_copy(i)
            for r in range(0, _LATE, 8):
                start(src.at[pl.ds(r, 8)], dst.at[pl.ds(r, 8)], s, 1)
        wait(*v_copy(LAST, 1))
        o_v[LAST] = normalise(o0, _dot(p_v[1], v_v[LAST, 1]), l_last)
        s_early = acc_v[...] + _dot_nt(o_v[LAST], woe_v[:, LAST * HW:HQD])
        o_ref[:, _LATE:D] = (x8[:, _LATE:D] + s_early * gate[:, _LATE:D])[0:2].astype(o_ref.dtype)

        for i in range(NL):
            c0, c1 = _LATE_CUTS[i], _LATE_CUTS[i + 1]
            lhs = jnp.concatenate([o_v[h] for h in range(c0 // HW, c1 // HW)], axis=1)
            wait(*late_copy(i))
            part = _dot_nt(lhs, wol_v[:, c0:c1])
            if i == 0:
                late_v[...] = part
            elif i < NL - 2:
                late_v[...] += part
            elif i == NL - 2:
                late_v[...] = x8[:, 0:_LATE] + (late_v[...] + part) * gate[:, 0:_LATE]
            else:
                o_ref[:, 0:_LATE] = (late_v[...] + part * gate[:, 0:_LATE])[0:2].astype(o_ref.dtype)

    return kernel, NSEM


@jax.jit
def pallas_recurrent_scan__sliding_block_cached__dense_activation_gelu__decode_kernel(
    A_x: jax.Array,
    A_k_cache: jax.Array,
    A_v_cache: jax.Array,
    A_wq: jax.Array,
    A_wo: jax.Array,
    B_x: jax.Array,
    B_w1: jax.Array,
    B_b1: jax.Array,
    B_w2: jax.Array,
    B_b2: jax.Array,
):
    del B_x
    B, SQ, D = A_x.shape
    _, HKV, SK, DH = A_k_cache.shape
    HQD = A_wq.shape[1]
    REP = HQD // DH // HKV
    F = B_w1.shape[1]
    W = min(4096, max(256, SK // 4))
    assert B == 2 and SQ == 1 and REP == 2 and F % 256 == 0
    HW = REP * DH

    kernel, nsem = _make_kernel(B, D, HKV, REP, SK, DH, W, F)
    hbm = pl.BlockSpec(memory_space=pl.ANY)
    out = pl.pallas_call(
        kernel,
        in_specs=[hbm] * 9,
        out_specs=pl.BlockSpec(memory_space=pltpu.VMEM),
        out_shape=jax.ShapeDtypeStruct((B, D), A_x.dtype),
        scratch_shapes=[
            pltpu.VMEM((B, D), _BF16),
            pltpu.VMEM((F // 128, 128), _BF16),
            pltpu.VMEM((D,), _BF16),
            pltpu.VMEM((D, HQD), _BF16),
            pltpu.VMEM((D - _LATE, HQD), _BF16),
            pltpu.VMEM((_LATE, HQD), _BF16),
            pltpu.VMEM((D, F), _BF16),
            pltpu.VMEM((D, F), _BF16),
            pltpu.VMEM((HKV, B, W, DH), _BF16),
            pltpu.VMEM((HKV, B, W, DH), _BF16),
            pltpu.VMEM((HKV, 8, DH), _BF16),
            pltpu.VMEM((2, 8, W), _BF16),
            pltpu.VMEM((HKV, 8, HW), _BF16),
            pltpu.VMEM((8, D - _LATE), _F32),
            pltpu.VMEM((8, _LATE), _F32),
            pltpu.SemaphoreType.DMA((nsem,)),
        ],
        compiler_params=pltpu.CompilerParams(
            vmem_limit_bytes=120 * 1024 * 1024,
            disable_semaphore_checks=True,
            disable_bounds_checks=True,
        ),
    )(
        A_x.reshape(B, D),
        A_k_cache,
        A_v_cache,
        A_wq,
        A_wo.T,
        B_w1,
        B_b1.reshape(F // 128, 128),
        B_w2.T,
        B_b2,
    )
    return out.reshape(B, SQ, D)
```

```python
import jax
import jax.numpy as jnp
from jax.experimental import pallas as pl
from jax.experimental.pallas import tpu as pltpu

_NT = (((1,), (1,)), ((), ()))
_F32 = jnp.float32
_BF16 = jnp.bfloat16

_KV_ROWS = 176
_KV_SKEW = 2
_LATE = 128
_LATE_CUTS = (0, 2048, 3072, 3584, 4096)


def _dot(a, b):
    return jnp.dot(a, b, preferred_element_type=_F32)


def _dot_nt(a, b):
    return jax.lax.dot_general(a, b, _NT, preferred_element_type=_F32)


def _make_kernel(B, D, HKV, REP, SK, DH, W, F):
    HW = REP * DH
    HQD = HKV * HW
    FT = F // 128
    scale = float(DH) ** -0.5
    LAST = HKV - 1
    EARLY = D - _LATE
    NL = len(_LATE_CUTS) - 1
    assert _LATE_CUTS[0] == 0 and _LATE_CUTS[-1] == HQD
    assert all(c % HW == 0 for c in _LATE_CUTS)
    S_X, S_B1, S_B2, S_WQ, S_W1, S_W2, S_WO = range(7)
    S_L = 7
    S_K = S_L + NL
    S_V = S_K + B * HKV
    NSEM = S_V + B * HKV

    def kernel(x_hbm, k_hbm, v_hbm, wq_hbm, wo_hbm, w1_hbm, b1_hbm, w2_hbm, b2_hbm,
               o_ref,
               x_v, b1_v, b2_v, wq_v, woe_v, wol_v, w1_v, w2_v, k_v, v_v,
               q_v, p_v, o_v, acc_v, late_v, sem):
        def start(src, dst, s, thread):
            pltpu.make_async_copy(src, dst, sem.at[s]).start(priority=thread)

        def wait(src, dst, s):
            pltpu.make_async_copy(src, dst, sem.at[s]).wait()

        def start_window(src, dst, s):
            half = W // 2
            pieces = [(r, min(_KV_ROWS, half - r)) for r in range(0, half, _KV_ROWS)]
            skewed = pieces[_KV_SKEW:] + pieces[:_KV_SKEW]
            for (r0, n0), (r1, n1) in zip(pieces, skewed):
                rows0, rows1 = pl.ds(r0, n0), pl.ds(half + r1, n1)
                start(src.at[rows0], dst.at[rows0], s, 0)
                start(src.at[rows1], dst.at[rows1], s, 1)

        def start_matrix(src, dst, s, nrows, ncols):
            half, cw = nrows // 2, ncols // 2

            def body(i, carry):
                for c in range(2):
                    cols = pl.ds(c * cw, cw)
                    for t in range(2):
                        rows = pl.ds(pl.multiple_of(t * half + i * 8, 8), 8)
                        start(src.at[rows, cols], dst.at[rows, cols], s, t)
                return carry

            jax.lax.fori_loop(0, half // 8, body, 0)

        win = pl.ds(SK - W, W)
        k_copy = lambda h, b: (k_hbm.at[b, h, win], k_v.at[h, b], S_K + h * B + b)
        v_copy = lambda h, b: (v_hbm.at[b, h, win], v_v.at[h, b], S_V + h * B + b)
        woe_copy = (wo_hbm.at[pl.ds(_LATE, EARLY)], woe_v, S_WO)

        def late_copy(i):
            cols = pl.ds(_LATE_CUTS[i], _LATE_CUTS[i + 1] - _LATE_CUTS[i])
            return wo_hbm.at[pl.ds(0, _LATE), cols], wol_v.at[:, cols], S_L + i

        def start_k(h):
            for b in range(B):
                start_window(*k_copy(h, b))

        def start_v(h):
            for b in range(B):
                start_window(*v_copy(h, b))

        start(x_hbm, x_v, S_X, 0)
        start(b1_hbm, b1_v, S_B1, 0)
        start(b2_hbm, b2_v, S_B2, 0)
        start_matrix(wq_hbm, wq_v, S_WQ, D, HQD)
        start_matrix(w1_hbm, w1_v, S_W1, D, F)

        wait(x_hbm, x_v, S_X)
        x2 = x_v[...].astype(_F32)
        row_d = jax.lax.broadcasted_iota(jnp.int32, (8, D), 0)
        x8 = jnp.where(row_d % 2 == 0,
                       jnp.broadcast_to(x2[0:1, :], (8, D)),
                       jnp.broadcast_to(x2[1:2, :], (8, D)))
        mean = jnp.mean(x8, axis=1, keepdims=True)
        xc = x8 - mean
        var = jnp.mean(xc * xc, axis=1, keepdims=True)
        xn = (xc / jnp.sqrt(var + 1e-5)).astype(_BF16)

        wait(wq_hbm, wq_v, S_WQ)
        q_all = _dot(xn, wq_v[...])
        row_h = jax.lax.broadcasted_iota(jnp.int32, (8, DH), 0)
        rep1 = (row_h // 2) % 2 == 1
        for h in range(HKV):
            q_v[h] = jnp.where(rep1,
                               q_all[:, h * HW + DH:(h + 1) * HW],
                               q_all[:, h * HW:h * HW + DH]).astype(_BF16)
        start_matrix(w2_hbm, w2_v, S_W2, D, F)

        wait(w1_hbm, w1_v, S_W1)
        wait(b1_hbm, b1_v, S_B1)
        b1f = b1_v[...].astype(_F32)
        bias1 = jnp.concatenate(
            [jnp.broadcast_to(b1f[t:t + 1, :], (8, 128)) for t in range(FT)], axis=1)
        hid = jax.nn.gelu(_dot(xn, w1_v[...]) + bias1, approximate=True).astype(_BF16)
        start_matrix(woe_copy[0], woe_v, S_WO, EARLY, HQD)
        wait(w2_hbm, w2_v, S_W2)
        wait(b2_hbm, b2_v, S_B2)
        y = _dot_nt(hid, w2_v[...]) + b2_v[...].astype(_F32).reshape(1, D)
        gate = y * jax.nn.sigmoid(y)

        start_k(0)
        start_k(1)
        start_v(0)
        start_k(2)
        start_v(1)

        batch1_w = jax.lax.broadcasted_iota(jnp.int32, (8, W), 0) % 2 == 1
        batch1_h = row_h % 2 == 1

        def scores(h):
            wait(*k_copy(h, 0))
            wait(*k_copy(h, 1))
            qh = q_v[h]
            s = jnp.where(batch1_w, _dot_nt(qh, k_v[h, 1]), _dot_nt(qh, k_v[h, 0]))
            m = jnp.max(s, axis=1, keepdims=True)
            p = jnp.exp((s - m) * scale)
            return p.astype(_BF16), jnp.sum(p, axis=1, keepdims=True)

        def normalise(o0, o1, l):
            o = jnp.where(batch1_h, o1, o0) / l
            return jnp.concatenate([o, pltpu.roll(o, 6, 0)], axis=1).astype(_BF16)

        def values(h, pb, l):
            wait(*v_copy(h, 0))
            wait(*v_copy(h, 1))
            o = normalise(_dot(pb, v_v[h, 0]), _dot(pb, v_v[h, 1]), l)
            o_v[h] = o
            col = h * HW if isinstance(h, int) else pl.multiple_of(h * HW, HW)
            acc_v[...] += _dot_nt(o, woe_v[:, pl.ds(col, HW)])

        def head(h, carry):
            values(h, *scores(h))
            start_k(h + 3)
            start_v(h + 2)
            return carry

        acc_v[...] = jnp.zeros_like(acc_v)
        wait(*woe_copy)
        jax.lax.fori_loop(0, HKV - 3, head, 0)

        values(HKV - 3, *scores(HKV - 3))
        pb, l_prev = scores(HKV - 2)
        p_v[0] = pb
        start_v(LAST)
        pb, l_last = scores(LAST)
        p_v[1] = pb
        values(HKV - 2, p_v[0], l_prev)
        wait(*v_copy(LAST, 0))
        o0 = _dot(p_v[1], v_v[LAST, 0])
        for i in range(NL):
            src, dst, s = late_copy(i)
            for r in range(0, _LATE, 8):
                start(src.at[pl.ds(r, 8)], dst.at[pl.ds(r, 8)], s, 1)
        wait(*v_copy(LAST, 1))
        o_v[LAST] = normalise(o0, _dot(p_v[1], v_v[LAST, 1]), l_last)
        s_early = acc_v[...] + _dot_nt(o_v[LAST], woe_v[:, LAST * HW:HQD])
        o_ref[:, _LATE:D] = (x8[:, _LATE:D] + s_early * gate[:, _LATE:D])[0:2].astype(o_ref.dtype)

        for i in range(NL):
            c0, c1 = _LATE_CUTS[i], _LATE_CUTS[i + 1]
            lhs = jnp.concatenate([o_v[h] for h in range(c0 // HW, c1 // HW)], axis=1)
            wait(*late_copy(i))
            part = _dot_nt(lhs, wol_v[:, c0:c1])
            if i == 0:
                late_v[...] = part
            elif i < NL - 2:
                late_v[...] += part
            elif i == NL - 2:
                late_v[...] = x8[:, 0:_LATE] + (late_v[...] + part) * gate[:, 0:_LATE]
            else:
                o_ref[:, 0:_LATE] = (late_v[...] + part * gate[:, 0:_LATE])[0:2].astype(o_ref.dtype)

    return kernel, NSEM


@jax.jit
def pallas_recurrent_scan__sliding_block_cached__dense_activation_gelu__decode_kernel(
    A_x: jax.Array,
    A_k_cache: jax.Array,
    A_v_cache: jax.Array,
    A_wq: jax.Array,
    A_wo: jax.Array,
    B_x: jax.Array,
    B_w1: jax.Array,
    B_b1: jax.Array,
    B_w2: jax.Array,
    B_b2: jax.Array,
):
    del B_x
    B, SQ, D = A_x.shape
    _, HKV, SK, DH = A_k_cache.shape
    HQD = A_wq.shape[1]
    REP = HQD // DH // HKV
    F = B_w1.shape[1]
    W = min(4096, max(256, SK // 4))
    assert B == 2 and SQ == 1 and REP == 2 and F % 256 == 0
    HW = REP * DH

    kernel, nsem = _make_kernel(B, D, HKV, REP, SK, DH, W, F)
    hbm = pl.BlockSpec(memory_space=pl.ANY)
    out = pl.pallas_call(
        kernel,
        in_specs=[hbm] * 9,
        out_specs=pl.BlockSpec(memory_space=pltpu.VMEM),
        out_shape=jax.ShapeDtypeStruct((B, D), A_x.dtype),
        scratch_shapes=[
            pltpu.VMEM((B, D), _BF16),
            pltpu.VMEM((F // 128, 128), _BF16),
            pltpu.VMEM((D,), _BF16),
            pltpu.VMEM((D, HQD), _BF16),
            pltpu.VMEM((D - _LATE, HQD), _BF16),
            pltpu.VMEM((_LATE, HQD), _BF16),
            pltpu.VMEM((D, F), _BF16),
            pltpu.VMEM((D, F), _BF16),
            pltpu.VMEM((HKV, B, W, DH), _BF16),
            pltpu.VMEM((HKV, B, W, DH), _BF16),
            pltpu.VMEM((HKV, 8, DH), _BF16),
            pltpu.VMEM((2, 8, W), _BF16),
            pltpu.VMEM((HKV, 8, HW), _BF16),
            pltpu.VMEM((8, D - _LATE), _F32),
            pltpu.VMEM((8, _LATE), _F32),
            pltpu.SemaphoreType.DMA((nsem,)),
        ],
        compiler_params=pltpu.CompilerParams(
            vmem_limit_bytes=120 * 1024 * 1024,
            disable_semaphore_checks=True,
            disable_bounds_checks=True,
        ),
    )(
        A_x.reshape(B, D),
        A_k_cache,
        A_v_cache,
        A_wq,
        A_wo.T,
        B_w1,
        B_b1.reshape(F // 128, 128),
        B_w2.T,
        B_b2,
    )
    return out.reshape(B, SQ, D)
```
